```python
import jax
import jax.numpy as jnp

def _softmax(x, axis=-1):
    return jax.nn.softmax(x, axis=axis)

def _gelu(x):
    return jax.nn.gelu(x, approximate=True)

def _silu(x):
    return jax.nn.silu(x)

def _sigmoid(x):
    return jax.nn.sigmoid(x)

def _layernorm(x, axis=-1, eps=1e-05):
    m = jnp.mean(x, axis=axis, keepdims=True)
    v = jnp.var(x, axis=axis, keepdims=True)
    return (x - m) / jnp.sqrt(v + eps)

def _scatter_add(tgt, idx, src, axis=0):
    return tgt.at[idx].add(src)

def _segment_sum(src, seg, n):
    return jax.ops.segment_sum(src, seg, n)

class _Rng:

    def __init__(self, key):
        self._k = key

    def _next(self):
        self._k, sub = jax.random.split(self._k)
        return sub

    def normal(self, shape):
        return jax.random.normal(self._next(), shape, dtype=jnp.bfloat16)

    def randint(self, lo, hi, shape):
        return jax.random.randint(self._next(), shape, lo, hi, dtype=jnp.int32)

    def uniform(self, shape, lo=0.0, hi=1.0):
        return jax.random.uniform(self._next(), shape, jnp.bfloat16, lo, hi)

    def permutation(self, n):
        return jax.random.permutation(self._next(), n)
kernel_name = 'adaLN_cond__memory_aug_recurrent_mem_tr__dense_activation_gelu__prompt'

def setup_inputs():
    _rng = _Rng(jax.random.key(int.from_bytes(__import__("os").urandom(4), "little")))
    _w = lambda a: (lambda t: t.astype(jnp.bfloat16) if jnp.issubdtype(t.dtype, jnp.floating) else t)(jnp.asarray(a))

    def _A_setup():
        B, S, Dm = (1, 2048, 1024)
        H, Dh = (32, 128)
        M, seg = (8, 32)
        seg = min(seg, S)
        S = S // seg * seg
        return {'x': _w((lambda *s: _rng.normal(s) * 0.05)(B, S, Dm)), 'mem0': _w((lambda *s: _rng.normal(s) * 0.05)(B, M, Dm)), 'Wq': _w((lambda *s: _rng.normal(s) * 0.05)(Dm, H, Dh) * Dm ** (-0.5)), 'Wk': _w((lambda *s: _rng.normal(s) * 0.05)(Dm, H, Dh) * Dm ** (-0.5)), 'Wv': _w((lambda *s: _rng.normal(s) * 0.05)(Dm, H, Dh) * Dm ** (-0.5)), 'Wo': _w((lambda *s: _rng.normal(s) * 0.05)(H, Dh, Dm) * (H * Dh) ** (-0.5)), 'seg_len': seg}
    _A_in = _A_setup()

    def _B_setup():
        B, S, D, F = (1, 2048, 1024, 3584)
        return {'x': _w((lambda *s: _rng.normal(s) * 0.05)(B, S, D)), 'w1': _w((lambda *s: _rng.normal(s) * 0.05)(D, F) * D ** (-0.5)), 'b1': _w((lambda *s: _rng.normal(s) * 0.05)(F) * 0.01), 'w2': _w((lambda *s: _rng.normal(s) * 0.05)(F, D) * F ** (-0.5)), 'b2': _w((lambda *s: _rng.normal(s) * 0.05)(D) * 0.01)}
    _B_in = _B_setup()
    return {'A_x': _A_in['x'], 'A_mem0': _A_in['mem0'], 'A_Wq': _A_in['Wq'], 'A_Wk': _A_in['Wk'], 'A_Wv': _A_in['Wv'], 'A_Wo': _A_in['Wo'], 'A_seg_len': _A_in['seg_len'], 'B_x': _B_in['x'], 'B_w1': _B_in['w1'], 'B_b1': _B_in['b1'], 'B_w2': _B_in['w2'], 'B_b2': _B_in['b2'], 'c': _w((lambda *s: _rng.normal(s) * 0.05)(1, 1024)), 'w_mod': _w((lambda *s: _rng.normal(s) * 0.05)(1024, 6 * 1024) * 1024 ** (-0.5))}

def reference(A_x, A_mem0, A_Wq, A_Wk, A_Wv, A_Wo, A_seg_len, B_x, B_w1, B_b1, B_w2, B_b2, c, w_mod):

    def _A_ref(x, mem0, Wq, Wk, Wv, Wo, seg_len):
        B, S, Dm = x.shape
        H, Dh = (Wq.shape[1], Wq.shape[2])
        M = mem0.shape[1]
        scale = Dh ** (-0.5)
        n_seg = S // seg_len
        L = M + seg_len
        idx = jnp.arange(L)
        mask = (idx[:, None] < M) | (idx[:, None] >= idx[None, :])
        mem = mem0
        outs = []
        for s in range(n_seg):
            xs = x[:, s * seg_len:(s + 1) * seg_len, :].copy()
            h = jnp.concatenate([mem, xs], axis=1)
            q = jnp.einsum('btd,dhe->bhte', h, Wq)
            k = jnp.einsum('btd,dhe->bhte', h, Wk)
            v = jnp.einsum('btd,dhe->bhte', h, Wv)
            scores = jnp.einsum('bhqe,bhke->bhqk', q, k) * scale
            scores = jnp.where(mask[None, None], scores, -1000000000.0)
            p = _softmax(scores, axis=-1)
            o = jnp.einsum('bhqk,bhke->bhqe', p, v)
            o = jnp.einsum('bhte,hed->btd', o, Wo)
            mem = o[:, :M, :].copy()
            outs.append(o[:, M:, :])
        return jnp.concatenate(outs, axis=1)

    def _B_ref(x, w1, b1, w2, b2):
        h = jnp.einsum('bsd,df->bsf', x, w1) + b1
        h = _gelu(h)
        return jnp.einsum('bsf,fd->bsd', h, w2) + b2
    x = A_x
    mod = (_silu(c) @ w_mod).reshape(c.shape[0], 6, 1, -1)
    sa, ca, ga, sb, cb, gb = (mod[:, 0].copy(), mod[:, 1].copy(), mod[:, 2].copy(), mod[:, 3].copy(), mod[:, 4].copy(), mod[:, 5].copy())
    h = _layernorm(x, axis=-1) * (1 + ca) + sa
    x = x + ga * _A_ref(h, A_mem0, A_Wq, A_Wk, A_Wv, A_Wo, A_seg_len)
    h = _layernorm(x, axis=-1) * (1 + cb) + sb
    x = x + gb * _B_ref(h, B_w1, B_b1, B_w2, B_b2)
    return x
```

```python
import functools

import jax
import jax.numpy as jnp
import jax.experimental.pallas as pl
import jax.experimental.pallas.tpu as pltpu

f32 = jnp.float32
bf16 = jnp.bfloat16
i32 = jnp.int32


def _dot(a, b):
    return jax.lax.dot_general(a, b, (((1,), (0,)), ((), ())), preferred_element_type=f32)


def _dott(a, b):
    return jax.lax.dot_general(a, b, (((1,), (1,)), ((), ())), preferred_element_type=f32)


def _bc(x):
    return pltpu.bitcast(x, bf16)


def _ln(x):
    m = jnp.mean(x, axis=-1, keepdims=True)
    d = x - m
    v = jnp.mean(d * d, axis=-1, keepdims=True)
    return d / jnp.sqrt(v + 1e-5)


def _kernel(x_hbm, mem_ref, wq_hbm, wk_hbm, wv_hbm, wo_hbm, w1_hbm, b1_ref, w2_hbm,
            b2_ref, c_ref, wm_hbm, o_hbm,
            xs, hs, wm, sq, sk, sv, so, tmp, wq, wk, wv, wo, w1, w2, mod,
            sx, sm, sw, sf, sout, *, S, D, H, SEG, M, F):
    NC = 8
    CD = D // NC
    CO = H * 128 // NC
    L = M + SEG

    def cpm(j):
        return pltpu.make_async_copy(wm_hbm.at[:, pl.ds(j * D, D)], wm.at[:, pl.ds(j * D, D)], sm.at[j])

    def cpw(a, i):
        if a < 3:
            src, dst, n = (wq_hbm, wk_hbm, wv_hbm)[a], (sq, sk, sv)[a], CD
        else:
            src, dst, n = wo_hbm, so, CO
        r = pl.ds(pl.multiple_of(i * n, n), n)
        return pltpu.make_async_copy(src.at[r], dst.at[r], sw.at[a * NC + i])

    cx = pltpu.make_async_copy(x_hbm, xs, sx)
    c1 = pltpu.make_async_copy(w1_hbm, w1, sf.at[0])
    c2 = pltpu.make_async_copy(w2_hbm, w2, sf.at[1])
    cpm(0).start(); cpm(1).start(); cx.start()
    for a in range(4):
        for i in range(NC):
            cpw(a, i).start()
    cpm(2).start()

    cv = c_ref[...].astype(f32)
    sc_ = jnp.broadcast_to(cv * jax.nn.sigmoid(cv), (8, D)).astype(bf16)

    def do_mod(j):
        cpm(j).wait()
        mod[j] = _dot(sc_, wm[:, j * D:(j + 1) * D])

    do_mod(0); do_mod(1)
    cx.wait()

    def ln1(i, _):
        r = pl.ds(pl.multiple_of(i * 128, 128), 128)
        h = _ln(xs[r, :].astype(f32)) * (1 + mod[1][:1]) + mod[0][:1]
        hs[r, :] = h.astype(bf16).astype(f32)
        return 0
    jax.lax.fori_loop(0, S // 128, ln1, 0)

    for a, (st, w) in enumerate(((sq, wq), (sk, wk), (sv, wv))):
        def rp(i, _, a=a, st=st, w=w):
            cpw(a, i).wait()
            v = pltpu.bitcast(st[pl.ds(pl.multiple_of(i * CD, CD), CD)], i32)
            v = v.reshape(CD // 2, 2, H // 2, 128)
            e = v[:, 0].reshape(CD // 2 * (H // 2), 128)
            o = v[:, 1].reshape(CD // 2 * (H // 2), 128)
            tmp[0] = (e & 0xFFFF) | (o << 16)
            tmp[1] = jax.lax.shift_right_logical(e, 16) | (o & jnp.int32(-65536))
            r = pl.ds(pl.multiple_of(i * (CD // 2), CD // 2), CD // 2)
            for j in range(H // 2):
                for p in range(2):
                    w[2 * j + p, r, :] = tmp[p, pl.ds(j, CD // 2, stride=H // 2), :]
            return 0
        jax.lax.fori_loop(0, NC, rp, 0)

    def rpo(i, _):
        cpw(3, i).wait()
        wo[pl.ds(pl.multiple_of(i * (CO // 2), CO // 2), CO // 2), :] = pltpu.bitcast(
            so[pl.ds(pl.multiple_of(i * CO, CO), CO), :], i32)
        return 0
    jax.lax.fori_loop(0, NC, rpo, 0)
    do_mod(2)
    for j in range(3, 6):
        cpm(j).start()
    c1.start(); c2.start()

    GH = 128 // L
    r = jax.lax.broadcasted_iota(i32, (GH * L, 128), 0)
    c = jax.lax.broadcasted_iota(i32, (GH * L, 128), 1)
    hr = sum((r >= k * L).astype(i32) for k in range(1, GH + 1))
    hc = sum((c >= k * L).astype(i32) for k in range(1, GH + 1))
    ri = r - L * hr
    cj = c - L * hc
    mask = (hr == hc) & ((ri < M) | (ri >= cj))
    G = [(g0, min(GH, H - g0)) for g0 in range(0, H, GH)]
    ga = mod[2][:1]
    scale = 128 ** -0.5

    def step(s, mem):
        rows = pl.ds(pl.multiple_of(s * SEG, SEG), SEG)
        hcat = jnp.concatenate([mem, hs[rows, :]], 0)

        def P(g):
            g0, n = G[g]
            return [[_dot(hcat, _bc(w[g0 + i])) for i in range(n)] for w in (wq, wk, wv)]

        def A1(g, qkv):
            n = G[g][1]
            q, k, v = qkv
            z = [jnp.zeros((128 - L * n, 128), f32)]
            k3 = jnp.concatenate(k + z, 0).astype(bf16)
            v3 = jnp.concatenate(v + z, 0).astype(bf16)
            sc = _dott(jnp.concatenate(q, 0), k3) * scale
            sc = jnp.where(mask[:L * n], sc, -1e9)
            e = jnp.exp(sc - sc.max(-1, keepdims=True))
            return e / e.sum(-1, keepdims=True), v3

        def A2(g, pv):
            o3 = _dot(*pv)
            return jnp.concatenate([o3[L * i:L * (i + 1)] for i in range(G[g][1])], 1)

        def O(g, oc):
            g0, n = G[g]
            return _dot(oc, _bc(wo[g0 * 64:(g0 + n) * 64, :]))

        N = len(G)
        st = {}
        acc = None
        for t in range(N + 3):
            if t < N:
                st['p', t] = P(t)
            if 0 <= t - 1 < N:
                st['a', t - 1] = A1(t - 1, st.pop(('p', t - 1)))
            if 0 <= t - 2 < N:
                st['b', t - 2] = A2(t - 2, st.pop(('a', t - 2)))
            if 0 <= t - 3 < N:
                y = O(t - 3, st.pop(('b', t - 3)))
                acc = y if acc is None else acc + y
        hs[rows, :] = xs[rows, :].astype(f32) + ga * acc[M:]
        return acc[:M].astype(bf16).astype(f32)
    jax.lax.fori_loop(0, S // SEG, step, mem_ref[...].astype(f32))

    c1.wait(); c2.wait()
    for j in range(3, 6):
        do_mod(j)
    BM = 256
    FC = 512

    def cpo(i):
        rr = pl.ds(pl.multiple_of(i * BM, BM), BM)
        return pltpu.make_async_copy(xs.at[rr], o_hbm.at[rr], sout.at[i])

    def mlp(i, _):
        rr = pl.ds(pl.multiple_of(i * BM, BM), BM)
        x1 = hs[rr, :]
        h = (_ln(x1) * (1 + mod[4][:1]) + mod[3][:1]).astype(bf16)
        acc = None
        for f0 in range(0, F, FC):
            u = _dot(h, w1[:, f0:f0 + FC]) + b1_ref[:, f0:f0 + FC].astype(f32)
            y = _dot(jax.nn.gelu(u, approximate=True).astype(bf16), w2[f0:f0 + FC, :])
            acc = y if acc is None else acc + y
        xs[rr, :] = (x1 + mod[5][:1] * (acc + b2_ref[...].astype(f32))).astype(bf16)
        cpo(i).start()
        return 0
    jax.lax.fori_loop(0, S // BM, mlp, 0)
    for i in range(S // BM):
        cpo(i).wait()


@functools.partial(jax.jit, static_argnames=("A_seg_len",))
def pallas_adaLN_cond__memory_aug_recurrent_mem_tr__dense_activation_gelu__prompt_kernel(
        A_x, A_mem0, A_Wq, A_Wk, A_Wv, A_Wo, A_seg_len, B_x, B_w1, B_b1, B_w2, B_b2, c, w_mod):
    B, S, D = A_x.shape
    H, Dh = A_Wq.shape[1:]
    M = A_mem0.shape[1]
    F = B_w1.shape[1]
    assert B == 1 and Dh == 128
    hb = pl.BlockSpec(memory_space=pl.ANY)
    vm = pl.BlockSpec(memory_space=pltpu.VMEM)
    V = pltpu.VMEM
    sem = pltpu.SemaphoreType.DMA
    out = pl.pallas_call(
        functools.partial(_kernel, S=S, D=D, H=H, SEG=A_seg_len, M=M, F=F),
        out_shape=jax.ShapeDtypeStruct((S, D), bf16),
        in_specs=[hb, vm, hb, hb, hb, hb, hb, vm, hb, vm, vm, hb],
        out_specs=hb,
        scratch_shapes=[
            V((S, D), bf16), V((S, D), f32), V((D, 6 * D), bf16),
            V((D, H, 128), bf16), V((D, H, 128), bf16), V((D, H, 128), bf16),
            V((H * 128, D), bf16), V((2, D // 16 * (H // 2), 128), i32),
            V((H, D // 2, 128), i32), V((H, D // 2, 128), i32), V((H, D // 2, 128), i32),
            V((H * 64, D), i32), V((D, F), bf16), V((F, D), bf16), V((6, 8, D), f32),
            sem, sem((6,)), sem((32,)), sem((2,)), sem((S // 256,)),
        ],
        compiler_params=pltpu.CompilerParams(vmem_limit_bytes=120 * 2**20),
    )(A_x.reshape(S, D), A_mem0.reshape(M, D), A_Wq, A_Wk, A_Wv, A_Wo.reshape(H * Dh, D),
      B_w1, B_b1.reshape(1, F), B_w2, B_b2.reshape(1, D), c, w_mod)
    return out.reshape(B, S, D)
```
